```python
import os as _os
_os.environ.setdefault("JAX_PLATFORMS", "cpu")
import jax
import jax.numpy as jnp

def _softmax(x, axis=-1):
    return jax.nn.softmax(x, axis=axis)
def _gelu(x):
    return jax.nn.gelu(x, approximate=True)
def _silu(x):
    return jax.nn.silu(x)
def _sigmoid(x):
    return jax.nn.sigmoid(x)
def _layernorm(x, axis=-1, eps=1e-5):
    m = jnp.mean(x, axis=axis, keepdims=True)
    v = jnp.var(x, axis=axis, keepdims=True)
    return (x - m) / jnp.sqrt(v + eps)
def _scatter_add(tgt, idx, src, axis=0):
    return tgt.at[idx].add(src)
def _segment_sum(src, seg, n):
    return jax.ops.segment_sum(src, seg, n)
class _Rng:
    def __init__(self, key):
        self._k = key
    def _next(self):
        self._k, sub = jax.random.split(self._k)
        return sub
    def normal(self, shape):
        return jax.random.normal(self._next(), shape, dtype=jnp.bfloat16)
    def randint(self, lo, hi, shape):
        return jax.random.randint(self._next(), shape, lo, hi, dtype=jnp.int32)
    def uniform(self, shape, lo=0.0, hi=1.0):
        return jax.random.uniform(self._next(), shape, jnp.bfloat16, lo, hi)
    def permutation(self, n):
        return jax.random.permutation(self._next(), n)


kernel_name = 'interleave_layers__grouped_kv_mqa__sliding_block__prompt'

def setup_inputs():
    _rng = _Rng(jax.random.key(int.from_bytes(__import__("os").urandom(4), "little")))
    _w = (lambda a: (lambda t: t.astype(jnp.bfloat16) if jnp.issubdtype(t.dtype, jnp.floating) else t)(jnp.asarray(a)))
    def _A_setup():
        B, S, D, H = 1, 2048, 448, 16
        Dh = D // H
        return {
            "x": _w((lambda *s: _rng.normal(s) * 0.05)(B, S, D)),
            "wq": _w((lambda *s: _rng.normal(s) * 0.05)(D, H * Dh)),
            "wk": _w((lambda *s: _rng.normal(s) * 0.05)(D, Dh)),
            "wv": _w((lambda *s: _rng.normal(s) * 0.05)(D, Dh)),
            "wo": _w((lambda *s: _rng.normal(s) * 0.05)(H * Dh, D)),
        }
    _A_in = _A_setup()

    def _B_setup():
        B, S, D = 1, 2048, 448
        return {
            "x": _w((lambda *s: _rng.normal(s) * 0.05)(B, S, D)),
            "wqkv": _w((lambda *s: _rng.normal(s) * 0.05)(D, 3 * D)),
            "wo": _w((lambda *s: _rng.normal(s) * 0.05)(D, D)),
        }
    _B_in = _B_setup()

    return {
        "A_x": _A_in["x"],
        "A_wq": _A_in["wq"],
        "A_wk": _A_in["wk"],
        "A_wv": _A_in["wv"],
        "A_wo": _A_in["wo"],
        "B_x": _B_in["x"],
        "B_wqkv": _B_in["wqkv"],
        "B_wo": _B_in["wo"],
    }

def reference(A_x, A_wq, A_wk, A_wv, A_wo, B_x, B_wqkv, B_wo):
    def _A_ref(x, wq, wk, wv, wo):
        B, S, D = x.shape
        H = 16
        Dh = D // H
        q = (lambda x, *d: x.transpose(*d))((x @ wq).reshape(B, S, H, Dh), 0, 2, 1, 3)
        k = x @ wk
        v = x @ wv
        scores = jnp.einsum("bhqd,bkd->bhqk", q, k) * (Dh ** -0.5)
        p = _softmax(scores, axis=-1)
        o = jnp.einsum("bhqk,bkd->bhqd", p, v)
        return (lambda x, *d: x.transpose(*d))(o, 0, 2, 1, 3).reshape(B, S, H * Dh) @ wo

    def _B_ref(x, wqkv, wo):
        B, S, D = x.shape
        H = 16; Dh = D // H; W = 256
        qkv = (lambda x, *d: x.transpose(*d))((x @ wqkv).reshape(B, S, 3, H, Dh), 2, 0, 3, 1, 4)
        q, k, v = qkv[0], qkv[1], qkv[2]
        scores = jnp.einsum("bhqd,bhkd->bhqk", q, k) * (Dh ** -0.5)
        idx = jnp.arange(S)
        mask = (idx[:, None] - idx[None, :] >= 0) & (idx[:, None] - idx[None, :] < W)
        scores = jnp.where(mask[None, None], scores, -1e9)
        p = _softmax(scores, axis=-1)
        o = jnp.einsum("bhqk,bhkd->bhqd", p, v)
        return (lambda x, *d: x.transpose(*d))(o, 0, 2, 1, 3).reshape(B, S, D) @ wo

    x = A_x
    x = x + _A_ref(_layernorm(x, axis=-1), A_wq, A_wk, A_wv, A_wo)
    x = x + _B_ref(_layernorm(x, axis=-1), B_wqkv, B_wo)
    x = x + _A_ref(_layernorm(x, axis=-1), A_wq, A_wk, A_wv, A_wo)
    x = x + _B_ref(_layernorm(x, axis=-1), B_wqkv, B_wo)
    return x
```

```python
import math

import jax
import jax.numpy as jnp
from jax import lax
import jax.experimental.pallas as pl
import jax.experimental.pallas.tpu as pltpu

S = 2048
D = 448
H = 16
DH = D // H
HP = 32
DP = H * HP
W = 256
BT = 512
NT = S // BT
QT = 128
NG = 4
EPS = 1e-5
QSCALE = (DH ** -0.5) * math.log2(math.e)

F32 = jnp.float32
BF16 = jnp.bfloat16


def _dot(a, b):
    return jnp.dot(a, b, preferred_element_type=F32)


def _head_rows(y, h):
    base = (h // 2) * 2 * DH
    if h % 2 == 0:
        return y[base:base + HP]
    return pltpu.roll(y[base + 2 * DH - HP:base + 2 * DH], DH, 0)


def _row_iota(n):
    return lax.broadcasted_iota(jnp.int32, (HP, n), 0)


def _zero_pad(blk):
    return jnp.where(_row_iota(blk.shape[1]) < DH, blk, 0.0)


def _ones_pad(blk):
    r = _row_iota(blk.shape[1])
    return jnp.where(r < DH, blk, jnp.where(r == DH, 1.0, 0.0))


def _layernorm_t(x):
    mu = jnp.sum(x, axis=0, keepdims=True) * (1.0 / D)
    xc = x - mu
    var = jnp.sum(xc * xc, axis=0, keepdims=True) * (1.0 / D)
    return (xc * lax.rsqrt(var + EPS)).astype(BF16)


def _colmax8(s):
    return jnp.max(s.reshape(s.shape[0] // 8, 8, s.shape[1]), axis=0)


def _kernel(xt_ref, wq_ref, wkt_ref, wvt_ref, woa_ref, wqkv_ref, wob_ref, out_ref,
            x_s, wa_s, woa_s, wb_s, wob_s, q_s, k_s, v_s, o_s, sa_s, sb_s, mb_s):
    wa_s[0:D, :] = wq_ref[...].astype(F32).T.astype(BF16)
    kv = jnp.concatenate(
        [wkt_ref[...].astype(F32), wvt_ref[...].astype(F32), jnp.zeros((8, D), F32)], axis=0)
    wa_s[D:DP, :] = kv.astype(BF16)
    for c in range(3):
        wb_s[c * D:(c + 1) * D, :] = wqkv_ref[:, c * D:(c + 1) * D].astype(F32).T.astype(BF16)
    for src, dst in ((woa_ref, woa_s), (wob_ref, wob_s)):
        w = src[...].astype(F32)
        wp = jnp.concatenate([_zero_pad(_head_rows(w, h)) for h in range(H)], axis=0)
        dst[...] = wp.T.astype(BF16)

    def tok(t):
        return pl.ds(pl.multiple_of(t * BT, BT), BT)

    def residual(t, wo_s):
        x = x_s[:, tok(t)] + _dot(wo_s[...], o_s[:, tok(t)])
        x_s[:, tok(t)] = x
        return x

    def project_a(t, x):
        y = _dot(wa_s[...], _layernorm_t(x))
        for h in range(H):
            q_s[h * HP:(h + 1) * HP, tok(t)] = (_head_rows(y, h) * QSCALE).astype(BF16)
        kt = _zero_pad(_head_rows(y, H)).astype(BF16)
        kt = jnp.concatenate([kt, jnp.zeros((128 - HP, BT), BF16)], axis=0)
        k_s[0, tok(t), :] = kt.T
        v_s[0:HP, tok(t)] = _ones_pad(_head_rows(y, H + 1)).astype(BF16)

    def project_b(t, x):
        xn = _layernorm_t(x)
        yq = _dot(wb_s[0:D, :], xn)
        for h in range(H):
            q_s[h * HP:(h + 1) * HP, tok(t)] = (_head_rows(yq, h) * QSCALE).astype(BF16)
        yk = _dot(wb_s[D:2 * D, :], xn)
        for g in range(NG):
            kt = jnp.concatenate([_zero_pad(_head_rows(yk, 4 * g + j)) for j in range(4)], axis=0)
            k_s[g, tok(t), :] = kt.astype(BF16).T
        yv = _dot(wb_s[2 * D:3 * D, :], xn)
        for h in range(H):
            v_s[h * HP:(h + 1) * HP, tok(t)] = _ones_pad(_head_rows(yv, h)).astype(BF16)

    nb = H * NT

    def attn_a():
        def rows(b):
            return pl.ds(pl.multiple_of((b // NT) * HP, HP), HP)

        def step(b, m_prev, consume, produce):
            if produce:
                qn = q_s[rows(b + 1), tok((b + 1) % NT)]
                m = jnp.full((8, BT), -jnp.inf, F32)
            acc = jnp.zeros((HP, BT), F32)
            for c in range(S // 128):
                sl = slice(c * 128, (c + 1) * 128)
                if consume:
                    p = jnp.exp2(sa_s[sl, :] - m_prev).astype(BF16)
                if produce:
                    s = _dot(k_s[0, sl, 0:HP], qn)
                    sa_s[sl, :] = s
                    m = jnp.maximum(m, _colmax8(s))
                if consume:
                    acc = acc + _dot(v_s[0:HP, sl], p)
            if consume:
                o = acc * (1.0 / acc[DH:DH + 1, :])
                o_s[rows(b), tok(b % NT)] = o.astype(BF16)
            if produce:
                return jnp.max(m, axis=0, keepdims=True)
            return None

        m0 = step(jnp.int32(-1), None, False, True)
        m_last = lax.fori_loop(0, nb - 1, lambda b, m: step(b, m, True, True), m0)
        step(jnp.int32(nb - 1), m_last, True, False)

    def attn_b():
        ri = lax.broadcasted_iota(jnp.int32, (QT, 4 * QT), 0)
        ci = lax.broadcasted_iota(jnp.int32, (QT, 4 * QT), 1) % QT
        old = ri > ci

        def qtile(i):
            return pl.ds(pl.multiple_of(i * QT, QT), QT)

        def krange(i, n):
            return pl.ds(pl.multiple_of((i - (n - 1)) * QT, QT), n * QT)

        def produce(i, g, n):
            q = q_s[g * 128:(g + 1) * 128, qtile(i)]
            z = jnp.zeros((HP, QT), BF16)
            rhs = jnp.concatenate(
                [jnp.concatenate([q[j * HP:(j + 1) * HP] if r == j else z for r in range(4)], axis=0)
                 for j in range(4)], axis=1)
            s = _dot(k_s[g, krange(i, n), :], rhs)
            if n == 3:
                sm = jnp.where(old, s[0:QT], s[2 * QT:])
            else:
                sm = jnp.where(old, -jnp.inf, s[(n - 1) * QT:])
            sb_s[g, 0:QT, :] = sm
            m = _colmax8(sm)
            if n > 1:
                s1 = s[(n - 2) * QT:(n - 1) * QT]
                sb_s[g, QT:, :] = s1
                m = jnp.maximum(m, _colmax8(s1))
            mb_s[g] = jnp.broadcast_to(jnp.max(m, axis=0, keepdims=True), (8, 4 * QT))

        def probs(g, n):
            m = mb_s[g, 0:1, :]
            pm = jnp.exp2(sb_s[g, 0:QT, :] - m)
            parts = []
            if n == 3:
                parts.append(jnp.where(old, pm, 0.0).astype(BF16))
            if n > 1:
                parts.append(jnp.exp2(sb_s[g, QT:, :] - m).astype(BF16))
            parts.append((jnp.where(old, 0.0, pm) if n == 3 else pm).astype(BF16))
            return jnp.concatenate(parts, axis=0) if n > 1 else parts[0]

        def consume(i, g, n, p):
            for j in range(4):
                r = slice(g * 128 + j * HP, g * 128 + (j + 1) * HP)
                acc = _dot(v_s[r, krange(i, n)], p[:, j * QT:(j + 1) * QT])
                o_s[r, qtile(i)] = (acc * (1.0 / acc[DH:DH + 1, :])).astype(BF16)

        def step(i, n_cur, n_nxt):
            for g in range(NG):
                if n_cur:
                    p = probs(g, n_cur)
                if n_nxt:
                    produce(i + 1, g, n_nxt)
                if n_cur:
                    consume(i, g, n_cur, p)

        step(jnp.int32(-1), 0, 1)
        step(jnp.int32(0), 1, 2)
        step(jnp.int32(1), 2, 3)

        def body(i, carry):
            step(i, 3, 3)
            return carry

        lax.fori_loop(2, S // QT - 1, body, 0)
        step(jnp.int32(S // QT - 1), 3, 0)

    def loop(fn):
        def body(t, carry):
            fn(t)
            return carry
        lax.fori_loop(0, NT, body, 0)

    def first(t):
        x = xt_ref[:, tok(t)].astype(F32)
        x_s[:, tok(t)] = x
        project_a(t, x)

    loop(first)

    def pair(l, carry):
        attn_a()
        loop(lambda t: project_b(t, residual(t, woa_s)))
        attn_b()

        @pl.when(l == 0)
        def _():
            loop(lambda t: project_a(t, residual(t, wob_s)))

        return carry

    lax.fori_loop(0, 2, pair, 0)

    def last(t):
        out_ref[:, tok(t)] = residual(t, wob_s).astype(out_ref.dtype)

    loop(last)


@jax.jit
def pallas_interleave_layers__grouped_kv_mqa__sliding_block__prompt_kernel(
    A_x: jax.Array,
    A_wq: jax.Array,
    A_wk: jax.Array,
    A_wv: jax.Array,
    A_wo: jax.Array,
    B_x: jax.Array,
    B_wqkv: jax.Array,
    B_wo: jax.Array,
):
    del B_x
    out_t = pl.pallas_call(
        _kernel,
        out_shape=jax.ShapeDtypeStruct((D, S), A_x.dtype),
        scratch_shapes=[
            pltpu.VMEM((D, S), F32),
            pltpu.VMEM((DP, D), BF16),
            pltpu.VMEM((D, DP), BF16),
            pltpu.VMEM((3 * D, D), BF16),
            pltpu.VMEM((D, DP), BF16),
            pltpu.VMEM((DP, S), BF16),
            pltpu.VMEM((NG, S, 128), BF16),
            pltpu.VMEM((DP, S), BF16),
            pltpu.VMEM((DP, S), BF16),
            pltpu.VMEM((S, BT), F32),
            pltpu.VMEM((NG, 2 * QT, 4 * QT), F32),
            pltpu.VMEM((NG, 8, 4 * QT), F32),
        ],
        compiler_params=pltpu.CompilerParams(vmem_limit_bytes=100 * 1024 * 1024),
        name="interleave_layers",
    )(A_x[0].T, A_wq, A_wk.T, A_wv.T, A_wo, B_wqkv, B_wo)
    return out_t.T[None]
```

```python
import math

import jax
import jax.numpy as jnp
from jax import lax
import jax.experimental.pallas as pl
import jax.experimental.pallas.tpu as pltpu

S = 2048
D = 448
H = 16
DH = D // H
HP = 32
DP = H * HP
W = 256
BT = 512
NT = S // BT
NL = BT // 128
NB = H * NT
QT = 128
GR = 4 * DH
EPS = 1e-5
QSCALE = (DH ** -0.5) * math.log2(math.e)

UA = 8
RV_HEAD = 192
RV = 192
VA, VL, PM, OFF, AHEAD, TC, B0, BS = 4, 2, 128, 48, 27, 3, 128, 32
FO = 2
LN0_AT = ((1,), (0, 2), (0,))
LNB_AT = (8, 11, 15, 18)
LNA_AT = (7, 9, 11, 13)
LNX_AT = (2, 5, 8, 11, 14, 16)
KEYS0_AT = ((), range(0, 21, 4), range(0, 21, 4), range(0, 16))
KEYS_AT = ((), range(14, 21), range(14, 21), range(0, 14))
SUM_AT = (2, 9)
TILE_ORDER = (2, 3, 4, 5, 0, 6, 1) + tuple(range(7, S // QT))
DB = 10
SCORE_BOUND = 60.0
VALUE_BOUND = 2.0 ** 40

F32 = jnp.float32
BF16 = jnp.bfloat16
U32 = jnp.uint32


def _dot(a, b):
    return jnp.dot(a, b, preferred_element_type=F32)


def _unpack(x):
    return pltpu.bitcast(x, BF16)


def _head_rows(y, j):
    base = (j // 2) * 2 * DH
    if j % 2 == 0:
        return y[base:base + HP]
    return pltpu.roll(y[base + 2 * DH - HP:base + 2 * DH], DH, 0)


def _row_iota(n):
    return lax.broadcasted_iota(jnp.int32, (HP, n), 0)


def _zero_pad(blk):
    return jnp.where(_row_iota(blk.shape[1]) < DH, blk, 0.0)


def _ones_pad(blk):
    r = _row_iota(blk.shape[1])
    return jnp.where(r < DH, blk, jnp.where(r == DH, 1.0, 0.0))


class _Moments:
    def __init__(self):
        self.shift = None

    def add(self, x):
        if self.shift is None:
            self.shift, self.s1, self.s2 = x[0:1], 0.0, 0.0
        x = (x - self.shift).reshape(x.shape[0] // 8, 8, x.shape[1])
        self.s1 = self.s1 + jnp.sum(x, axis=0)
        self.s2 = self.s2 + jnp.sum(x * x, axis=0)

    def result(self):
        d = jnp.sum(self.s1, axis=0, keepdims=True) * (1.0 / D)
        var = jnp.sum(self.s2, axis=0, keepdims=True) * (1.0 / D) - d * d
        return self.shift + d, lax.rsqrt(jnp.maximum(var, 0.0) + EPS)


def _colmax8(s):
    return jnp.max(s.reshape(s.shape[0] // 8, 8, s.shape[1]), axis=0)


def _normalize(acc):
    return acc * (1.0 / acc[DH:DH + 1, :])


def _left_operands(a11, a12, a21, a22):
    return a11 + a12, a21 + a22, a11, a22, a11 + a22, a12 - a22, a21 - a11


def _right_operands(b11, b12, b21, b22):
    return b22, b11, b12 - b22, b21 - b11, b11 + b22, b21 + b22, b11 + b12


def _strassen(product):
    m5, m2, m3 = product(0), product(1), product(2)
    c12, c22 = m3 + m5, m3 - m2
    m4 = product(3)
    c21, c11 = m2 + m4, m4 - m5
    m1 = product(4)
    c11, c22 = c11 + m1, c22 + m1
    c11 = c11 + product(5)
    c22 = c22 + product(6)
    return jnp.concatenate([c11, c12], axis=1), jnp.concatenate([c21, c22], axis=1)


def _run(gen):
    for _ in gen:
        pass


def _kernel(xt_hbm, wq_hbm, wkt_hbm, wvt_hbm, woa_hbm, wqkv_hbm, wob_hbm, out_hbm,
            xin_s, wq_in, wkt_in, wvt_in, woa_in, wqkv_in, wob_in, out_s,
            wa_s, woa_s, wb_s, wob_s, xn_s, q_s, ka_s, kb_s, v_s, o_s, p_s, s_s, qtab_s, ktab0_s, ktab1_s,
            sems, *bufs):
    xs, pa = bufs[:NT], bufs[NT:]
    ka32, kb32, p32 = ka_s.bitcast(U32), kb_s.bitcast(U32), p_s.bitcast(U32)
    xn32, q32, v32, o32 = (r.bitcast(U32) for r in (xn_s, q_s, v_s, o_s))

    def load_tiles(ref32, tile0, n, row0, rows):
        if not isinstance(row0, int):
            sl = pl.ds(pl.multiple_of(row0 // 2, rows // 2), rows // 2)
        else:
            sl = slice(row0 // 2, (row0 + rows) // 2)
        return jnp.concatenate([_unpack(ref32[tile0 + l, sl, :]) for l in range(n)], axis=1)

    def store_tiles(ref, tile0, row0, val):
        if not isinstance(row0, int):
            sl = pl.ds(pl.multiple_of(row0, val.shape[0]), val.shape[0])
        else:
            sl = slice(row0, row0 + val.shape[0])
        for l in range(val.shape[1] // 128):
            ref[tile0 + l, sl, :] = val[:, l * 128:(l + 1) * 128].astype(BF16)

    def tok(t):
        return slice(t * BT, (t + 1) * BT)

    x_in = [pltpu.make_async_copy(xt_hbm.at[:, tok(t)], xin_s.at[0:D, tok(t)], sems.at[t])
            for t in range(NT)]
    x_out = [pltpu.make_async_copy(out_s.at[:, tok(t)], out_hbm.at[:, tok(t)], sems.at[NT + t])
             for t in range(NT)]
    w_in = [pltpu.make_async_copy(src, dst, sems.at[2 * NT + n]) for n, (src, dst) in enumerate((
        (wkt_hbm, wkt_in), (wvt_hbm, wvt_in), (wq_hbm, wq_in),
        (woa_hbm, woa_in), (wob_hbm, wob_in), (wqkv_hbm, wqkv_in)))]

    def store_left(dst, r0, lo, hi):
        n = lo.shape[0] // 2
        for i, w in enumerate(_left_operands(lo[:n], hi[:n], lo[n:], hi[n:])):
            if w.shape[1] % 128:
                w = jnp.concatenate([w, jnp.zeros((n, -w.shape[1] % 128), F32)], axis=1)
            store_tiles(dst, 0, r0 + i * n, w)

    def prep(src, dst):
        for u in range(src.shape[1] // (2 * GR)):
            w = src[:, u * 2 * GR:(u + 1) * 2 * GR].astype(F32)
            half = w.shape[0] // 2
            lo = w[:half].T
            yield
            store_left(dst, u * 7 * GR, lo, w[half:].T)
            yield

    def prep_kv():
        z = jnp.zeros((HP - DH, D), F32)
        w = jnp.concatenate([wkt_in[...].astype(F32), z, wvt_in[...].astype(F32), z], axis=0)
        store_left(wa_s, 14 * GR, w[:, :D // 2], w[:, D // 2:])

    def prep_wo():
        for src, dst in ((woa_in, woa_s), (wob_in, wob_s)):
            for c in range(0, D, 128):
                w = src[:, c:min(c + 128, D)].astype(F32)
                w = jnp.concatenate([_zero_pad(_head_rows(w, h)) for h in range(H)], axis=0)
                store_tiles(dst, 0, c, w.T)
                yield

    def prep_wb():
        yield from prep(wqkv_in, wb_s)
        kb_s[:, 0:3 * HP, :] = jnp.zeros((H, 3 * HP, 128), BF16)

    def hrows(h):
        return slice(h * HP, (h + 1) * HP)

    def matmul(w_s, r0, rows, right, hook):
        def product(i):
            b = right(i)
            y = _dot(load_tiles(w_s.bitcast(U32), 0, 2, r0 + i * rows, rows)[:, 0:b.shape[0]], b)
            hook(y)
            return y
        return _strassen(product)

    def paced(*jobs):
        count = [0]
        for gen, _ in jobs:
            next(gen)

        def hook(y):
            for gen, at in jobs:
                if count[0] in at:
                    gen.send(y)
            count[0] += 1
        return hook

    def unpaced(gen, n):
        while True:
            yield
            for _ in range(n):
                next(gen, None)

    def forward(gen):
        while True:
            gen.send((yield))

    def load_x(t, stats):
        moments = _Moments()
        for r in range(0, D, D // 2):
            y = yield
            if y is not None:
                xin_s[pl.ds(pl.multiple_of(D + 16 * zero, 16), 16), 0:128] = (
                    y[0:16, 0:128].astype(xin_s.dtype))
            for c in range(r, r + D // 2, 16):
                x = xin_s[c:c + 16, tok(t)].astype(F32)
                xs[t][c:c + 16, :] = x
                moments.add(x)
        stats[t] = moments.result()
        yield from layernorm(t, stats)

    def layernorm(t, stats):
        n = D // 2
        for l in range(2):
            for r in range(0, n, n // 2):
                y = yield
                if y is not None:
                    xs[t][pl.ds(pl.multiple_of(D + 8 * zero, 8), 8), 0:128] = y[0:8, 0:128]
                mu, scale = stats[t]
                for c in range(r, r + n // 2, 16):
                    quarters = []
                    for r0 in (c, n + c):
                        for cols in (slice(l * 128, (l + 1) * 128), slice((l + 2) * 128, (l + 3) * 128)):
                            quarters.append((xs[t][r0:r0 + 16, cols] - mu[:, cols]) * scale[:, cols])
                    for i, b in enumerate(_right_operands(*quarters)):
                        store_tiles(xn_s, (t * 7 + i) * 2 + l, c, b)
        yield

    def normalized(t):
        return lambda i: load_tiles(xn32, (t * 7 + i) * 2, 2, 0, D // 2)

    def add_out_proj(t, wo_s, hook, emit):
        o = load_tiles(o32, t * NL, NL, 0, DP)
        moments = _Moments()
        for g in range(D // GR):
            y = _dot(load_tiles(wo_s.bitcast(U32), 0, DP // 128, g * GR, GR), o)
            hook(y)
            for c in range(0, GR, 16):
                rows = slice(g * GR + c, g * GR + c + 16)
                x = xs[t][rows, :] + y[c:c + 16]
                xs[t][rows, :] = x
                moments.add(x)
                if emit:
                    out_s[rows, tok(t)] = x.astype(out_s.dtype)
        return moments.result()

    def q_proj(t, u, w_s, hook):
        heads = []
        for g, y in enumerate(matmul(w_s, u * 7 * GR, GR, normalized(t), hook), 2 * u):
            for j in range(4):
                heads.append(_head_rows(y, j) * QSCALE)
                store_tiles(q_s, t * NL, (4 * g + j) * HP, heads[-1])
        return heads

    ktabs = (ktab0_s, ktab1_s)
    spare = DH * RV // 8

    def spread_k():
        k = ka_s[0:RV, :].astype(F32)
        for d in range(DH):
            spread = jnp.broadcast_to(k[:, d:d + 1], (RV, 128)).reshape(RV // 8, 8, 128)
            for ktab in ktabs:
                ktab[d * RV // 8:(d + 1) * RV // 8] = spread
            yield

    def project_a(t, hook):
        kt, v = matmul(wa_s, 14 * GR, HP, normalized(t), hook)
        ka_s[tok(t), :] = jnp.concatenate(
            [kt.astype(BF16), jnp.zeros((128 - HP, BT), BF16)], axis=0).T
        v = _ones_pad(v)
        store_tiles(v_s, t * NL, 0, v)
        qq = None
        for u in range(2):
            for q in q_proj(t, u, wa_s, hook):
                n = jnp.sum(q * q, axis=0, keepdims=True)
                qq = n if qq is None else jnp.maximum(qq, n)
        return qq, jnp.sum(kt * kt, axis=0, keepdims=True), _colmax8(jnp.abs(v))

    def no_shift_needed(bounds):
        qq, kk, vv = (jnp.max(jnp.concatenate(b, axis=0)) for b in zip(*bounds))
        return jnp.logical_and(qq * kk <= SCORE_BOUND ** 2, vv <= VALUE_BOUND)

    def store_window_keys(t, g, y):
        kt = jnp.concatenate([_zero_pad(_head_rows(y, j)) for j in range(4)], axis=0)
        k = pltpu.bitcast(kt.astype(BF16).T, U32)
        rolled = [k] + [pltpu.roll(k, HP * s, 1) for s in range(1, 4)]
        n, m = BT // 2, HP // 2
        lane = lax.broadcasted_iota(jnp.int32, (n - 3 * m, 128), 1)
        r0 = t * n + 3 * m
        for j in range(4):
            part = [rolled[(lg - j) % 4] for lg in range(4)]
            row = part[0][0:n - 3 * m]
            for lg in range(1, 4):
                row = jnp.where(lane >= lg * HP, part[lg][lg * m:n - (3 - lg) * m], row)
            kb32[4 * g + j, r0:r0 + n - 3 * m, :] = row
            for lg in range(4):
                lanes = slice(lg * HP, (lg + 1) * HP)
                if lg > 0:
                    kb32[4 * g + j, r0 - lg * m:r0, lanes] = part[lg][0:lg * m, lanes]
                if lg < 3:
                    kb32[4 * g + j, r0 + n - 3 * m:r0 + n - lg * m, lanes] = (
                        part[lg][n - (3 - lg) * m:n, lanes])

    def project_b(t, hook):
        for u in range(2):
            for g, y in enumerate(matmul(wb_s, (2 + u) * 7 * GR, GR, normalized(t), hook), 2 * u):
                store_window_keys(t, g, y)
            for g, y in enumerate(matmul(wb_s, (4 + u) * 7 * GR, GR, normalized(t), hook), 2 * u):
                for j in range(4):
                    store_tiles(v_s, t * NL, (4 * g + j) * HP, _ones_pad(_head_rows(y, j)))
            q_proj(t, u, wb_s, hook)

    def load_q(b):
        b = min(b, NB - 1) if isinstance(b, int) else jnp.minimum(b, NB - 1)
        return load_tiles(q32, (b // H) * NL, NL, (b % H) * HP, HP)

    def store_o(b, acc):
        store_tiles(o_s, (b // H) * NL, (b % H) * HP, _normalize(acc))

    def keys(lo, hi):
        return _unpack(ka32[lo // 2:hi // 2, :])[:, 0:HP]

    def put_probs(u, lo, l0, s):
        p = jnp.exp2(s)
        for l in range(s.shape[1] // 128):
            pa[u][l0 + l, lo:lo + s.shape[0], :] = p[:, l * 128:(l + 1) * 128].astype(BF16)

    def stage_q(b):
        q = load_q(b).astype(F32)
        for r in range(HP // 8):
            for l in range(NL):
                ktab0_s[spare + 1 + r * NL + l] = q[r * 8:(r + 1) * 8, l * 128:(l + 1) * 128]

    def spread_q(u, d):
        for l in range(NL):
            q = ktab0_s[spare + 1 + (d // 8) * NL + l]
            qtab_s[(u * DH + d) * NL + l] = jnp.broadcast_to(q[d % 8:d % 8 + 1, :], (8, 128))

    def a_steps(b0, finish, start, rv):
        work = [(u, r0, l0, d) for u in range(UA) for r0 in range(0, rv // 8, VA)
                for l0 in range(0, NL, VL) for d in range(DH)]
        done, batch, accs = 0, 0, [None] * VA
        for u in range(UA):
            old32 = pa[u].bitcast(U32)
            acc, lo, nd = None, rv, 0
            if start:
                qn = load_q(b0 + u + UA)
                stage_q(b0 + u + UA + 1)
            for c in range(S // 128):
                if finish:
                    p = jnp.concatenate(
                        [_unpack(old32[l, c * 64:(c + 1) * 64, :]) for l in range(NL)], axis=1)
                    part = _dot(load_tiles(v32, c, 1, 0, HP), p)
                    acc = part if acc is None else acc + part
                while start and lo < (c + 1) * 128:
                    hi = (lo // PM + 1) * PM
                    s = _dot(keys(lo, hi), qn)
                    for r in range(0, hi - lo, 16):
                        put_probs(u, lo + r, 0, s[r:r + 16])
                        n = lo + r + 16 - rv
                        if n >= B0 and n % BS == 0 and nd < DH:
                            spread_q((u + 1) % UA, nd)
                            nd += 1
                        due = min(len(work) * (u * (S - rv) + n) // (UA * (S - rv) - OFF),
                                  (u + 1) * len(work) // UA + AHEAD, len(work))
                        if due > done:
                            batch += 1
                            ktabs[batch % 2][spare + zero] = s[r:r + 8, TC * 128:(TC + 1) * 128]
                        while done < due:
                            wu, r0, l0, d = work[done]
                            done += 1
                            qb = jnp.concatenate(
                                [qtab_s[(wu * DH + d) * NL + l0 + l] for l in range(VL)], axis=1)
                            for a in range(VA):
                                kb = ktabs[batch % 2][d * RV // 8 + r0 + a]
                                term = jnp.concatenate([kb] * VL, axis=1) * qb
                                accs[a] = term if d == 0 else accs[a] + term
                            if d == DH - 1:
                                put_probs(wu, 8 * r0, l0, jnp.concatenate(accs, axis=0))
                    lo = hi
            if finish:
                store_o(b0 + u, acc)
            assert not start or nd == DH
        assert not start or done == len(work)

    def a_unshifted():
        stage_q(0)
        for d in range(DH):
            spread_q(0, d)
        a_steps(-UA, False, True, RV_HEAD)

        def body(i, carry):
            a_steps(i * UA, True, True, RV)
            return carry
        lax.fori_loop(0, NB // UA - 1, body, 0)
        a_steps(NB - UA, True, False, RV)

    def a_shifted():
        def body(b, carry):
            qn = load_q(b)
            m = None
            for c in range(NT):
                s = _dot(keys(c * BT, (c + 1) * BT), qn)
                s_s[tok(c), :] = s
                m = _colmax8(s) if m is None else jnp.maximum(m, _colmax8(s))
            m = jnp.max(m, axis=0, keepdims=True)

            def chunk(c, acc):
                p = jnp.exp2(s_s[pl.ds(pl.multiple_of(c * 256, 256), 256), :] - m).astype(BF16)
                return acc + _dot(load_tiles(v32, 2 * c, 2, 0, HP), p)

            store_o(b, lax.fori_loop(0, S // 256, chunk, jnp.zeros((HP, BT), F32)))
            return carry
        lax.fori_loop(0, NB, body, 0)

    nb = W // HP

    def b_scores(i, h):
        row = lax.broadcasted_iota(jnp.int32, (HP, QT), 0)
        col = lax.broadcasted_iota(jnp.int32, (HP, QT), 1)
        q = load_tiles(q32, i, 1, h * HP, HP).astype(F32)
        rhs = jnp.concatenate([jnp.where(col >> 5 == lg, q, 0.0) for lg in range(4)], axis=0)
        first = max(0, nb - 4 * i - 3)
        r0 = i * QT - W + first * HP + 3 * HP
        s = _dot(_unpack(kb32[h, r0 // 2:(r0 + (nb + 1 - first) * HP) // 2, :]), rhs.astype(BF16))
        blk = {n: s[(n - first) * HP:(n - first + 1) * HP] for n in range(first, nb + 1)}
        for n in range(first, nb - 4 * i):
            blk[n] = jnp.where((col >> 5) + n >= nb - 4 * i, blk[n], -jnp.inf)
        blk[nb] = jnp.where(row > (col & 31), blk.pop(0) if first == 0 else -jnp.inf, blk[nb])
        m = None
        for x in blk.values():
            m = _colmax8(x) if m is None else jnp.maximum(m, _colmax8(x))
        return blk, jnp.max(m, axis=0, keepdims=True)

    def b_finish(i, h, blk, m):
        p = {n: jnp.exp2(x - m) for n, x in blk.items()}
        if 4 * i >= nb:
            row = lax.broadcasted_iota(jnp.int32, (HP, QT), 0)
            old = row > (lax.broadcasted_iota(jnp.int32, (HP, QT), 1) & 31)
            p[0] = jnp.where(old, p[nb], 0.0)
            p[nb] = jnp.where(old, 0.0, p[nb])
        for n, x in p.items():
            p_s[h, hrows(n), :] = x.astype(BF16)
        p = {n: p32[h, n * HP // 2:(n + 1) * HP // 2, :] for n in p}
        zero = jnp.zeros((HP // 2, QT), U32)
        col = lax.broadcasted_iota(jnp.int32, (HP // 2, QT), 1)
        lo = max(0, nb - 4 * i)
        c = {n: jnp.where(col & HP != 0, p.get(n - 1, zero), p.get(n, zero))
             for n in range(max(0, lo - 2), nb + 2)}
        u = [jnp.where(col & (2 * HP) != 0, c.get(n - 2, zero), c.get(n, zero))
             for n in range(lo, nb + 4)]
        tiles = (nb + 4 - lo) // 4
        acc = _dot(load_tiles(v32, i + 1 - tiles, tiles, h * HP, HP),
                   _unpack(jnp.concatenate(u, axis=0)))
        store_tiles(o_s, i, h * HP, _normalize(acc))

    def b_attention():
        pending = []
        for i in TILE_ORDER:
            for h in range(H):
                pending.append((i, h) + b_scores(i, h))
                if len(pending) > DB:
                    b_finish(*pending.pop(0))
                yield
        while pending:
            b_finish(*pending.pop(0))
            yield

    def add_attention(wo_s, extra_jobs, emit):
        stats = {}
        ln = layernorm(0, stats)
        next(ln)
        for t in range(NT):
            jobs = extra_jobs[t] + ([(forward(ln), LN0_AT[t - 1])] if t else [])
            stats[t] = add_out_proj(t, wo_s, paced(*jobs), emit)
            if emit:
                for cp in ([], [], x_out[:3], x_out[3:])[t]:
                    cp.start()
        return stats

    def next_layernorm(t, stats, at):
        return [(layernorm(t + 1, stats), at)] if t + 1 < NT else []

    for cp in x_in[:1] + w_in[:3]:
        cp.start()
    x_in[0].wait()
    for cp in x_in[1:]:
        cp.start()
    _run(load_x(0, {}))
    for cp in w_in[:3]:
        cp.wait()
    for cp in w_in[3:]:
        cp.start()
    zero = jnp.minimum(jnp.max(pltpu.bitcast(jnp.abs(wkt_in[0:16, :].astype(F32)), jnp.int32)), 0)
    prep_kv()
    keys0, bounds0 = spread_k(), []
    for t in range(NT):
        for cp in (x_in[1:2], x_in[2:], [], w_in[3:5])[t]:
            cp.wait()
        jobs = [(unpaced(keys0, 1), KEYS0_AT[t]) if t else (unpaced(prep(wq_in, wa_s), 2), (0, 7))]
        if t + 1 < NT:
            jobs.append((load_x(t + 1, {}), LNX_AT))
        else:
            jobs.append((unpaced(prep_wo(), 1), range(1, 17, 2)))
        bounds0.append(project_a(t, paced(*jobs)))
    _run(keys0)
    w_in[5].wait()

    def pair(l, safe):
        lax.cond(safe != 0, a_unshifted, a_shifted)
        weights = prep_wb()
        stats = add_attention(
            woa_s, [[(unpaced(weights, 1), range(4))] for _ in range(NT)], False)
        _run(weights)
        for t in range(NT):
            project_b(t, paced(*next_layernorm(t, stats, LNB_AT)))
        window = b_attention()
        for _ in range(H * S // QT + DB - 4 * FO):
            next(window)
        stats = add_attention(wob_s, [[(unpaced(window, FO), range(4))], [], [], []], True)

        def again():
            keys = spread_k()
            bounds = []
            for t in range(NT):
                jobs = [(unpaced(keys, 1), KEYS_AT[t])] + next_layernorm(t, stats, LNA_AT)
                bounds.append(project_a(t, paced(*jobs)))
            _run(keys)
            for cp in x_out:
                cp.wait()
            return no_shift_needed(bounds).astype(jnp.int32)

        return lax.cond(l == 0, again, lambda: safe)

    lax.fori_loop(0, 2, pair, no_shift_needed(bounds0).astype(jnp.int32))
    for cp in x_out:
        cp.wait()


@jax.jit
def pallas_interleave_layers__grouped_kv_mqa__sliding_block__prompt_kernel(
    A_x: jax.Array,
    A_wq: jax.Array,
    A_wk: jax.Array,
    A_wv: jax.Array,
    A_wo: jax.Array,
    B_x: jax.Array,
    B_wqkv: jax.Array,
    B_wo: jax.Array,
):
    del B_x
    operands = (A_x[0].T, A_wq, A_wk.T, A_wv.T, A_wo, B_wqkv, B_wo)
    out_t = pl.pallas_call(
        _kernel,
        out_shape=jax.ShapeDtypeStruct((D, S), A_x.dtype),
        in_specs=[pl.BlockSpec(memory_space=pl.ANY)] * len(operands),
        out_specs=pl.BlockSpec(memory_space=pl.ANY),
        scratch_shapes=[pltpu.VMEM((D + 16, S), A_x.dtype)]
        + [pltpu.VMEM(a.shape, a.dtype) for a in operands[1:]] + [
            pltpu.VMEM((D, S), A_x.dtype),
            pltpu.VMEM((2, 14 * GR + 7 * HP, 128), BF16),
            pltpu.VMEM((4, D, 128), BF16),
            pltpu.VMEM((2, 42 * GR, 128), BF16),
            pltpu.VMEM((4, D, 128), BF16),
            pltpu.VMEM((NT * 14, D // 2, 128), BF16),
            pltpu.VMEM((S // 128, DP, 128), BF16),
            pltpu.VMEM((S, 128), BF16),
            pltpu.VMEM((H, S + 3 * HP, 128), BF16),
            pltpu.VMEM((S // 128, DP, 128), BF16),
            pltpu.VMEM((S // 128, DP, 128), BF16),
            pltpu.VMEM((H, W + HP, QT), BF16),
            pltpu.VMEM((S, BT), F32),
            pltpu.VMEM((UA * DH * NL, 8, 128), F32),
            pltpu.VMEM((DH * RV // 8 + 1 + HP // 8 * NL, 8, 128), F32),
            pltpu.VMEM((DH * RV // 8 + 1, 8, 128), F32),
            pltpu.SemaphoreType.DMA((2 * NT + 6,)),
        ] + [pltpu.VMEM((D + 8, BT), F32)] * NT
        + [pltpu.VMEM((NL, S, 128), BF16)] * UA,
        compiler_params=pltpu.CompilerParams(vmem_limit_bytes=110 * 1024 * 1024),
        name="interleave_layers",
    )(*operands)
    return out_t.T[None]
```

```python
import math

import jax
import jax.numpy as jnp
from jax import lax
import jax.experimental.pallas as pl
import jax.experimental.pallas.tpu as pltpu

S = 2048
D = 448
H = 16
DH = D // H
HP = 32
DP = H * HP
W = 256
BT = 512
NT = S // BT
NL = BT // 128
NB = H * NT
QT = 128
GR = 4 * DH
EPS = 1e-5
QSCALE = (DH ** -0.5) * math.log2(math.e)

SCORE_BOUND = 60.0
VALUE_BOUND = 2.0 ** 40

UA = 8
RV = 192
VA, VL = 2, 4
DB = 10
TILE_ORDER = (2, 3, 0, 1) + tuple(range(4, S // QT))

F32 = jnp.float32
BF16 = jnp.bfloat16
U32 = jnp.uint32


def _dot(a, b):
    return jnp.dot(a, b, preferred_element_type=F32)


def _unpack(x):
    return pltpu.bitcast(x, BF16)


def _head_rows(y, j):
    base = (j // 2) * 2 * DH
    if j % 2 == 0:
        return y[base:base + HP]
    return pltpu.roll(y[base + 2 * DH - HP:base + 2 * DH], DH, 0)


def _zero_pad(blk):
    return jnp.where(lax.broadcasted_iota(jnp.int32, blk.shape, 0) < DH, blk, 0.0)


def _ones_pad(blk):
    r = lax.broadcasted_iota(jnp.int32, blk.shape, 0)
    return jnp.where(r < DH, blk, jnp.where(r == DH, 1.0, 0.0))


class _Moments:
    def __init__(self):
        self.shift = None

    def add(self, x):
        if self.shift is None:
            self.shift, self.s1, self.s2 = x[0:1], 0.0, 0.0
        x = (x - self.shift).reshape(x.shape[0] // 8, 8, x.shape[1])
        self.s1 = self.s1 + jnp.sum(x, axis=0)
        self.s2 = self.s2 + jnp.sum(x * x, axis=0)

    def result(self):
        d = jnp.sum(self.s1, axis=0, keepdims=True) * (1.0 / D)
        var = jnp.sum(self.s2, axis=0, keepdims=True) * (1.0 / D) - d * d
        return self.shift + d, lax.rsqrt(jnp.maximum(var, 0.0) + EPS)


def _colmax8(s):
    return jnp.max(s.reshape(s.shape[0] // 8, 8, s.shape[1]), axis=0)


def _normalize(acc):
    return acc * (1.0 / acc[DH:DH + 1, :])


def _left_operands(a11, a12, a21, a22):
    return a11 + a12, a21 + a22, a11, a22, a11 + a22, a12 - a22, a21 - a11


def _right_operands(b11, b12, b21, b22):
    return b22, b11, b12 - b22, b21 - b11, b11 + b22, b21 + b22, b11 + b12


def _strassen(product):
    m5, m2, m3 = product(0), product(1), product(2)
    c12, c22 = m3 + m5, m3 - m2
    m4 = product(3)
    c21, c11 = m2 + m4, m4 - m5
    m1 = product(4)
    c11, c22 = c11 + m1, c22 + m1
    c11 = c11 + product(5)
    c22 = c22 + product(6)
    return jnp.concatenate([c11, c12], axis=1), jnp.concatenate([c21, c22], axis=1)


def _paced(*jobs):
    count = [0]
    for job, _ in jobs:
        next(job)

    def hook(y):
        for job, at in jobs:
            if count[0] in at:
                job.send(y)
        count[0] += 1
    return hook


def _pieces(gen, n):
    while True:
        yield
        for _ in range(n):
            next(gen, None)


def _forward(job):
    while True:
        job.send((yield))


def _run(gen):
    for _ in gen:
        pass


def _kernel(xt_hbm, wq_hbm, wkt_hbm, wvt_hbm, woa_hbm, wqkv_hbm, wob_hbm, out_hbm,
            xin_s, wq_in, wkt_in, wvt_in, woa_in, wqkv_in, wob_in, out_s,
            wa_s, woa_s, wb_s, wob_s, xn_s, q_s, ka_s, kb_s, v_s, o_s, p_s, s_s, bound_s,
            qtab_s, ktab0_s, ktab1_s, sems, *bufs):
    xs, pa = bufs[:NT], bufs[NT:]
    ka32, kb32, p32 = ka_s.bitcast(U32), kb_s.bitcast(U32), p_s.bitcast(U32)
    xn32, q32, v32, o32 = (r.bitcast(U32) for r in (xn_s, q_s, v_s, o_s))

    def load_tiles(ref32, tile0, n, row0, rows):
        if isinstance(row0, int):
            sl = slice(row0 // 2, (row0 + rows) // 2)
        else:
            sl = pl.ds(pl.multiple_of(row0 // 2, rows // 2), rows // 2)
        return jnp.concatenate([_unpack(ref32[tile0 + l, sl, :]) for l in range(n)], axis=1)

    def store_tiles(ref, tile0, row0, val):
        if isinstance(row0, int):
            sl = slice(row0, row0 + val.shape[0])
        else:
            sl = pl.ds(pl.multiple_of(row0, val.shape[0]), val.shape[0])
        for l in range(val.shape[1] // 128):
            ref[tile0 + l, sl, :] = val[:, l * 128:(l + 1) * 128].astype(BF16)

    def tok(t):
        return slice(t * BT, (t + 1) * BT)

    x_in = [pltpu.make_async_copy(xt_hbm.at[:, tok(t)], xin_s.at[0:D, tok(t)], sems.at[t])
            for t in range(NT)]
    x_out = [pltpu.make_async_copy(out_s.at[:, tok(t)], out_hbm.at[:, tok(t)], sems.at[NT + t])
             for t in range(NT)]
    w_in = [pltpu.make_async_copy(src, dst, sems.at[2 * NT + n]) for n, (src, dst) in enumerate((
        (wkt_hbm, wkt_in), (wvt_hbm, wvt_in), (wq_hbm, wq_in),
        (woa_hbm, woa_in), (wob_hbm, wob_in), (wqkv_hbm, wqkv_in)))]

    def store_left(dst, r0, lo, hi):
        n = lo.shape[0] // 2
        for i, w in enumerate(_left_operands(lo[:n], hi[:n], lo[n:], hi[n:])):
            w = jnp.concatenate([w, jnp.zeros((n, -w.shape[1] % 128), F32)], axis=1)
            store_tiles(dst, 0, r0 + i * n, w)

    def prep(src, dst):
        for u in range(src.shape[1] // (2 * GR)):
            w = src[:, u * 2 * GR:(u + 1) * 2 * GR].astype(F32)
            lo = w[:D // 2].T
            yield
            store_left(dst, u * 7 * GR, lo, w[D // 2:].T)
            yield

    def prep_kv():
        z = jnp.zeros((HP - DH, D), F32)
        w = jnp.concatenate([wkt_in[...].astype(F32), z, wvt_in[...].astype(F32), z], axis=0)
        store_left(wa_s, 14 * GR, w[:, :D // 2], w[:, D // 2:])

    def prep_wo():
        for src, dst in ((woa_in, woa_s), (wob_in, wob_s)):
            for c in range(0, D, 128):
                w = src[:, c:min(c + 128, D)].astype(F32)
                w = jnp.concatenate([_zero_pad(_head_rows(w, h)) for h in range(H)], axis=0)
                store_tiles(dst, 0, c, w.T)
                yield

    def project(w_s, r0, rows, t, hook):
        def product(i):
            b = load_tiles(xn32, (t * 7 + i) * 2, 2, 0, D // 2)
            y = _dot(load_tiles(w_s.bitcast(U32), 0, 2, r0 + i * rows, rows)[:, 0:D // 2], b)
            hook(y)
            return y
        return _strassen(product)

    def load_x(t):
        moments = _Moments()
        for r in range(0, D, D // 2):
            y = yield
            if y is not None:
                xin_s[pl.ds(pl.multiple_of(D + 16 * zero, 16), 16), 0:128] = (
                    y[0:16, 0:128].astype(xin_s.dtype))
            for c in range(r, r + D // 2, 16):
                x = xin_s[c:c + 16, tok(t)].astype(F32)
                xs[t][c:c + 16, :] = x
                moments.add(x)
        yield from layernorm(t, {t: moments.result()})

    def layernorm(t, stats):
        n = D // 2
        for l in range(2):
            for r in range(0, n, n // 2):
                y = yield
                if y is not None:
                    xs[t][pl.ds(pl.multiple_of(D + 8 * zero, 8), 8), 0:128] = y[0:8, 0:128]
                mean, scale = stats[t]
                for c in range(r, r + n // 2, 16):
                    quarters = []
                    for r0 in (c, n + c):
                        for c0 in (l * 128, (l + 2) * 128):
                            cols = slice(c0, c0 + 128)
                            quarters.append(
                                (xs[t][r0:r0 + 16, cols] - mean[:, cols]) * scale[:, cols])
                    for i, b in enumerate(_right_operands(*quarters)):
                        store_tiles(xn_s, (t * 7 + i) * 2 + l, c, b)
        yield

    def add_out_proj(t, wo_s, hook, emit):
        o = load_tiles(o32, t * NL, NL, 0, DP)
        moments = _Moments()
        for g in range(D // GR):
            y = _dot(load_tiles(wo_s.bitcast(U32), 0, DP // 128, g * GR, GR), o)
            hook(y)
            for c in range(0, GR, 16):
                rows = slice(g * GR + c, g * GR + c + 16)
                x = xs[t][rows, :] + y[c:c + 16]
                xs[t][rows, :] = x
                moments.add(x)
                if emit:
                    out_s[rows, tok(t)] = x.astype(out_s.dtype)
        return moments.result()

    def q_proj(t, u, w_s, hook):
        heads = []
        for g, y in enumerate(project(w_s, u * 7 * GR, GR, t, hook), 2 * u):
            for j in range(4):
                heads.append(_head_rows(y, j) * QSCALE)
                store_tiles(q_s, t * NL, (4 * g + j) * HP, heads[-1])
        return heads

    def project_a(t, hook):
        kt, v = project(wa_s, 14 * GR, HP, t, hook)
        ka_s[tok(t), :] = jnp.concatenate(
            [kt.astype(BF16), jnp.zeros((128 - HP, BT), BF16)], axis=0).T
        v = _ones_pad(v)
        store_tiles(v_s, t * NL, 0, v)
        qq = None
        for u in range(2):
            for q in q_proj(t, u, wa_s, hook):
                n = jnp.sum(q * q, axis=0, keepdims=True)
                qq = n if qq is None else jnp.maximum(qq, n)
        return qq, jnp.sum(kt * kt, axis=0, keepdims=True), _colmax8(jnp.abs(v))

    def store_bounds(bounds):
        for i, b in enumerate(zip(*bounds)):
            b = jnp.concatenate(b, axis=0)
            bound_s[i] = jnp.broadcast_to(jnp.max(b, axis=0, keepdims=True), (8, BT))

    def no_shift_needed():
        qq, kk, vv = (jnp.max(bound_s[i]) for i in range(3))
        return jnp.logical_and(qq * kk <= SCORE_BOUND ** 2, vv <= VALUE_BOUND)

    def store_window_keys(t, g, y, earlier):
        kt = jnp.concatenate([_zero_pad(_head_rows(y, j)) for j in range(4)], axis=0)
        k = pltpu.bitcast(kt.astype(BF16).T, U32)
        n, m = BT // 2, HP // 2
        rolled = [k] + [pltpu.roll(k, HP * s, 1) for s in range(1, 4)]
        before = earlier.get(g, [jnp.zeros((3 * m, 128), U32)] * 4)
        earlier[g] = [x[n - 3 * m:] for x in rolled]
        rolled = [jnp.concatenate(pair, axis=0) for pair in zip(before, rolled)]
        lane = lax.broadcasted_iota(jnp.int32, (n, 128), 1)
        for j in range(4):
            rows = rolled[-j % 4][0:n]
            for lg in range(1, 4):
                rows = jnp.where(lane >= lg * HP, rolled[(lg - j) % 4][lg * m:lg * m + n], rows)
            kb32[4 * g + j, t * n:(t + 1) * n, :] = rows

    def project_b(t, hook, earlier):
        for u in range(2):
            for g, y in enumerate(project(wb_s, (2 + u) * 7 * GR, GR, t, hook), 2 * u):
                store_window_keys(t, g, y, earlier)
            for g, y in enumerate(project(wb_s, (4 + u) * 7 * GR, GR, t, hook), 2 * u):
                for j in range(4):
                    store_tiles(v_s, t * NL, (4 * g + j) * HP, _ones_pad(_head_rows(y, j)))
            q_proj(t, u, wb_s, hook)

    ktabs = (ktab0_s, ktab1_s)
    spare = DH * RV // 8

    def spread_k():
        k = ka_s[0:RV, :].astype(F32)
        for d in range(DH):
            spread = jnp.broadcast_to(k[:, d:d + 1], (RV, 128)).reshape(RV // 8, 8, 128)
            for ktab in ktabs:
                ktab[d * RV // 8:(d + 1) * RV // 8] = spread
            yield

    def load_q(b):
        b = min(b, NB - 1) if isinstance(b, int) else jnp.minimum(b, NB - 1)
        return load_tiles(q32, (b // H) * NL, NL, (b % H) * HP, HP)

    def store_o(b, acc):
        store_tiles(o_s, (b // H) * NL, (b % H) * HP, _normalize(acc))

    def keys(lo, hi):
        return _unpack(ka32[lo // 2:hi // 2, :])[:, 0:HP]

    def put_probs(u, lo, l0, s):
        p = jnp.exp2(s)
        for l in range(s.shape[1] // 128):
            pa[u][l0 + l, lo:lo + s.shape[0], :] = p[:, l * 128:(l + 1) * 128].astype(BF16)

    def stage_q(b):
        q = load_q(b).astype(F32)
        for r in range(HP // 8):
            for l in range(NL):
                ktab0_s[spare + 1 + r * NL + l] = q[r * 8:(r + 1) * 8, l * 128:(l + 1) * 128]

    def spread_q(u, d):
        for l in range(NL):
            q = ktab0_s[spare + 1 + (d // 8) * NL + l]
            qtab_s[(u * DH + d) * NL + l] = jnp.broadcast_to(q[d % 8:d % 8 + 1, :], (8, 128))

    def a_steps(b0, finish, start):
        work = [(u, r0, l0, d) for u in range(UA) for r0 in range(0, RV // 8, VA)
                for l0 in range(0, NL, VL) for d in range(DH)]
        done, batch, dots = 0, 0, None
        for u in range(UA):
            old32 = pa[u].bitcast(U32)
            acc, lo, nd = None, RV, 0
            if start:
                qn = load_q(b0 + u + UA)
                stage_q(b0 + u + UA + 1)
            for c in range(S // 128):
                if finish:
                    p = jnp.concatenate(
                        [_unpack(old32[l, c * 64:(c + 1) * 64, :]) for l in range(NL)], axis=1)
                    part = _dot(load_tiles(v32, c, 1, 0, HP), p)
                    acc = part if acc is None else acc + part
                hi = (c + 1) * 128
                if not start or hi <= lo:
                    continue
                s = _dot(keys(lo, hi), qn)
                for r in range(0, hi - lo, 16):
                    put_probs(u, lo + r, 0, s[r:r + 16])
                    n = lo + r + 16 - RV
                    if n >= 64 and n % 48 == 0 and nd < DH:
                        spread_q((u + 1) % UA, nd)
                        nd += 1
                    due = len(work) * (u * (S - RV) + n) // (UA * (S - RV))
                    if due > done:
                        batch += 1
                        ktabs[batch % 2][spare + zero] = s[r:r + 8, 256:384]
                    while done < due:
                        wu, r0, l0, d = work[done]
                        done += 1
                        qb = jnp.concatenate(
                            [qtab_s[(wu * DH + d) * NL + l0 + l] for l in range(VL)], axis=1)
                        k0 = d * RV // 8 + r0
                        kb = ktabs[batch % 2][k0:k0 + VA].reshape(VA * 8, 128)
                        term = (jnp.concatenate([kb] * VL, axis=1)
                                * jnp.concatenate([qb] * VA, axis=0))
                        dots = term if d == 0 else dots + term
                        if d == DH - 1:
                            put_probs(wu, 8 * r0, l0, dots)
                lo = hi
            if finish:
                store_o(b0 + u, acc)
            assert not start or nd == DH
        assert not start or done == len(work)

    def a_first_steps():
        stage_q(0)
        for d in range(DH):
            spread_q(0, d)
        a_steps(-UA, False, True)

    def a_unshifted():
        def body(i, carry):
            a_steps(i * UA, True, True)
            return carry
        lax.fori_loop(0, NB // UA - 1, body, 0)
        a_steps(NB - UA, True, False)

    def a_shifted():
        def body(b, carry):
            qn = load_q(b)
            m = None
            for c in range(NT):
                s = _dot(keys(c * BT, (c + 1) * BT), qn)
                s_s[tok(c), :] = s
                m = _colmax8(s) if m is None else jnp.maximum(m, _colmax8(s))
            m = jnp.max(m, axis=0, keepdims=True)

            def chunk(c, acc):
                p = jnp.exp2(s_s[pl.ds(pl.multiple_of(c * 256, 256), 256), :] - m).astype(BF16)
                return acc + _dot(load_tiles(v32, 2 * c, 2, 0, HP), p)

            store_o(b, lax.fori_loop(0, S // 256, chunk, jnp.zeros((HP, BT), F32)))
            return carry
        lax.fori_loop(0, NB, body, 0)

    nb = W // HP

    def b_scores(i, h):
        row = lax.broadcasted_iota(jnp.int32, (HP, QT), 0)
        col = lax.broadcasted_iota(jnp.int32, (HP, QT), 1)
        q = load_tiles(q32, i, 1, h * HP, HP).astype(F32)
        rhs = jnp.concatenate([jnp.where(col >> 5 == lg, q, 0.0) for lg in range(4)], axis=0)
        first = max(0, nb - 4 * i - 3)
        r0 = i * QT - W + first * HP + 3 * HP
        s = _dot(_unpack(kb32[h, r0 // 2:(r0 + (nb + 1 - first) * HP) // 2, :]), rhs.astype(BF16))
        blk = {n: s[(n - first) * HP:(n - first + 1) * HP] for n in range(first, nb + 1)}
        for n in range(first, nb - 4 * i):
            blk[n] = jnp.where((col >> 5) + n >= nb - 4 * i, blk[n], -jnp.inf)
        blk[nb] = jnp.where(row > (col & 31), blk.pop(0) if first == 0 else -jnp.inf, blk[nb])
        m = None
        for x in blk.values():
            m = _colmax8(x) if m is None else jnp.maximum(m, _colmax8(x))
        return blk, jnp.max(m, axis=0, keepdims=True)

    def b_finish(i, h, blk, m):
        p = {n: jnp.exp2(x - m) for n, x in blk.items()}
        if 4 * i >= nb:
            row = lax.broadcasted_iota(jnp.int32, (HP, QT), 0)
            old = row > (lax.broadcasted_iota(jnp.int32, (HP, QT), 1) & 31)
            p[0] = jnp.where(old, p[nb], 0.0)
            p[nb] = jnp.where(old, 0.0, p[nb])
        for n, x in p.items():
            p_s[h, n * HP:(n + 1) * HP, :] = x.astype(BF16)
        p = {n: p32[h, n * HP // 2:(n + 1) * HP // 2, :] for n in p}
        none = jnp.zeros((HP // 2, QT), U32)
        col = lax.broadcasted_iota(jnp.int32, (HP // 2, QT), 1)
        lo = max(0, nb - 4 * i)
        c = {n: jnp.where(col & HP != 0, p.get(n - 1, none), p.get(n, none))
             for n in range(max(0, lo - 2), nb + 2)}
        u = [jnp.where(col & (2 * HP) != 0, c.get(n - 2, none), c.get(n, none))
             for n in range(lo, nb + 4)]
        tiles = (nb + 4 - lo) // 4
        acc = _dot(load_tiles(v32, i + 1 - tiles, tiles, h * HP, HP),
                   _unpack(jnp.concatenate(u, axis=0)))
        store_tiles(o_s, i, h * HP, _normalize(acc))

    def b_attention():
        pending = []
        for i in TILE_ORDER:
            for h in range(H):
                pending.append((i, h) + b_scores(i, h))
                if len(pending) > DB:
                    b_finish(*pending.pop(0))
                yield
        while pending:
            b_finish(*pending.pop(0))
            yield

    def add_attention(wo_s, jobs, emit):
        stats = {}
        ln = layernorm(0, stats)
        next(ln)
        for t in range(NT):
            at = ((), (1,), (0, 2), (0,))[t]
            hook = _paced(*jobs[t], *([(_forward(ln), at)] if at else []))
            stats[t] = add_out_proj(t, wo_s, hook, emit)
            if emit:
                for cp in ([], [], x_out[:3], x_out[3:])[t]:
                    cp.start()
        return stats

    def next_layernorm(t, stats, at):
        return [(layernorm(t + 1, stats), at)] if t + 1 < NT else []

    for cp in x_in[:1] + w_in[:3]:
        cp.start()
    x_in[0].wait()
    for cp in x_in[1:]:
        cp.start()
    _run(load_x(0))
    for cp in w_in[:3]:
        cp.wait()
    for cp in w_in[3:]:
        cp.start()
    zero = jnp.minimum(jnp.max(pltpu.bitcast(jnp.abs(wkt_in[0:16, :].astype(F32)), jnp.int32)), 0)
    prep_kv()
    first_keys, first_bounds = spread_k(), []
    for t in range(NT):
        for cp in (x_in[1:2], x_in[2:], [], w_in[3:5])[t]:
            cp.wait()
        one = ((_pieces(prep(wq_in, wa_s), 2), (0, 7)) if t == 0 else
               (_pieces(first_keys, 1), range(0, 21, 4) if t + 1 < NT else range(16)))
        two = ((load_x(t + 1), (2, 4, 7, 10, 13, 16)) if t + 1 < NT else
               (_pieces(prep_wo(), 1), range(1, 17, 2)))
        first_bounds.append(project_a(t, _paced(one, two)))
    _run(first_keys)
    store_bounds(first_bounds)
    w_in[5].wait()

    def layer_pair(l, carry):
        safe = no_shift_needed()
        a_first_steps()
        lax.cond(safe, a_unshifted, a_shifted)
        weights = prep(wqkv_in, wb_s)
        stats = add_attention(woa_s, [[(_pieces(weights, 1), range(4))] for _ in range(NT)], False)
        _run(weights)
        earlier = {}
        for t in range(NT):
            project_b(t, _paced(*next_layernorm(t, stats, (8, 15, 29, 36))), earlier)
        window = b_attention()
        for _ in range(H * S // QT + DB - 8):
            next(window)
        stats = add_attention(wob_s, [[(_pieces(window, 2), range(4))], [], [], []], True)

        @pl.when(l == 0)
        def _():
            spread, bounds = spread_k(), []
            for t in range(NT):
                at = ((), range(14, 21), range(14, 21), range(14))[t]
                bounds.append(project_a(t, _paced(
                    (_pieces(spread, 1), at), *next_layernorm(t, stats, (7, 9, 11, 13)))))
            _run(spread)
            for cp in x_out:
                cp.wait()
            store_bounds(bounds)

        return carry

    lax.fori_loop(0, 2, layer_pair, 0)
    for cp in x_out:
        cp.wait()


@jax.jit
def pallas_interleave_layers__grouped_kv_mqa__sliding_block__prompt_kernel(
    A_x: jax.Array,
    A_wq: jax.Array,
    A_wk: jax.Array,
    A_wv: jax.Array,
    A_wo: jax.Array,
    B_x: jax.Array,
    B_wqkv: jax.Array,
    B_wo: jax.Array,
):
    del B_x
    operands = (A_x[0].T, A_wq, A_wk.T, A_wv.T, A_wo, B_wqkv, B_wo)
    scratch = [pltpu.VMEM((D + 16, S), A_x.dtype)]
    scratch += [pltpu.VMEM(a.shape, a.dtype) for a in operands[1:]]
    scratch += [
        pltpu.VMEM((D, S), A_x.dtype),
        pltpu.VMEM((2, 14 * GR + 7 * HP, 128), BF16),
        pltpu.VMEM((4, D, 128), BF16),
        pltpu.VMEM((2, 42 * GR, 128), BF16),
        pltpu.VMEM((4, D, 128), BF16),
        pltpu.VMEM((NT * 14, D // 2, 128), BF16),
        pltpu.VMEM((S // 128, DP, 128), BF16),
        pltpu.VMEM((S, 128), BF16),
        pltpu.VMEM((H, S, 128), BF16),
        pltpu.VMEM((S // 128, DP, 128), BF16),
        pltpu.VMEM((S // 128, DP, 128), BF16),
        pltpu.VMEM((H, W + HP, QT), BF16),
        pltpu.VMEM((S, BT), F32),
        pltpu.VMEM((3, 8, BT), F32),
        pltpu.VMEM((UA * DH * NL, 8, 128), F32),
        pltpu.VMEM((DH * RV // 8 + 1 + HP // 8 * NL, 8, 128), F32),
        pltpu.VMEM((DH * RV // 8 + 1, 8, 128), F32),
        pltpu.SemaphoreType.DMA((2 * NT + 6,)),
    ]
    scratch += [pltpu.VMEM((D + 8, BT), F32)] * NT
    scratch += [pltpu.VMEM((NL, S, 128), BF16)] * UA
    out_t = pl.pallas_call(
        _kernel,
        out_shape=jax.ShapeDtypeStruct((D, S), A_x.dtype),
        in_specs=[pl.BlockSpec(memory_space=pl.ANY)] * len(operands),
        out_specs=pl.BlockSpec(memory_space=pl.ANY),
        scratch_shapes=scratch,
        compiler_params=pltpu.CompilerParams(vmem_limit_bytes=100 * 1024 * 1024),
        name="interleave_layers",
    )(*operands)
    return out_t.T[None]
```

```python
import math

import jax
import jax.numpy as jnp
from jax import lax
import jax.experimental.pallas as pl
import jax.experimental.pallas.tpu as pltpu

S = 2048
D = 448
H = 16
DH = D // H
HP = 32
DP = H * HP
W = 256
BT = 512
NT = S // BT
NL = BT // 128
NB = H * NT
QT = 128
GR = 4 * DH
EPS = 1e-5
QSCALE = (DH ** -0.5) * math.log2(math.e)

SCORE_BOUND = 60.0
VALUE_BOUND = 2.0 ** 40

UA = 8
RV = 192
VA, VL = 2, 4
DB = 10
TILE_ORDER = (2, 3, 0, 1) + tuple(range(4, S // QT))

F32 = jnp.float32
BF16 = jnp.bfloat16
U32 = jnp.uint32


def _dot(a, b):
    return jnp.dot(a, b, preferred_element_type=F32)


def _unpack(x):
    return pltpu.bitcast(x, BF16)


def _head_rows(y, j):
    base = (j // 2) * 2 * DH
    if j % 2 == 0:
        return y[base:base + HP]
    return pltpu.roll(y[base + 2 * DH - HP:base + 2 * DH], DH, 0)


def _zero_pad(blk):
    return jnp.where(lax.broadcasted_iota(jnp.int32, blk.shape, 0) < DH, blk, 0.0)


def _ones_pad(blk):
    r = lax.broadcasted_iota(jnp.int32, blk.shape, 0)
    return jnp.where(r < DH, blk, jnp.where(r == DH, 1.0, 0.0))


class _Moments:
    def __init__(self):
        self.shift = None

    def add(self, x):
        if self.shift is None:
            self.shift, self.s1, self.s2 = x[0:1], 0.0, 0.0
        x = (x - self.shift).reshape(x.shape[0] // 8, 8, x.shape[1])
        self.s1 = self.s1 + jnp.sum(x, axis=0)
        self.s2 = self.s2 + jnp.sum(x * x, axis=0)

    def result(self):
        d = jnp.sum(self.s1, axis=0, keepdims=True) * (1.0 / D)
        var = jnp.sum(self.s2, axis=0, keepdims=True) * (1.0 / D) - d * d
        return self.shift + d, lax.rsqrt(jnp.maximum(var, 0.0) + EPS)


def _colmax8(s):
    return jnp.max(s.reshape(s.shape[0] // 8, 8, s.shape[1]), axis=0)


def _normalize(acc):
    return acc * (1.0 / acc[DH:DH + 1, :])


def _left_operands(a11, a12, a21, a22):
    return a11 + a12, a21 + a22, a11, a22, a11 + a22, a12 - a22, a21 - a11


def _right_operands(b11, b12, b21, b22):
    return b22, b11, b12 - b22, b21 - b11, b11 + b22, b21 + b22, b11 + b12


def _strassen(product):
    m5, m2, m3 = product(0), product(1), product(2)
    c12, c22 = m3 + m5, m3 - m2
    m4 = product(3)
    c21, c11 = m2 + m4, m4 - m5
    m1 = product(4)
    c11, c22 = c11 + m1, c22 + m1
    c11 = c11 + product(5)
    c22 = c22 + product(6)
    return jnp.concatenate([c11, c12], axis=1), jnp.concatenate([c21, c22], axis=1)


def _paced(*jobs):
    count = [0]
    for job, _ in jobs:
        next(job)

    def hook(y):
        for job, at in jobs:
            if count[0] in at:
                job.send(y)
        count[0] += 1
    return hook


def _pieces(gen, n):
    while True:
        yield
        for _ in range(n):
            next(gen, None)


def _forward(job):
    while True:
        job.send((yield))


def _run(gen):
    for _ in gen:
        pass


def _kernel(xt_hbm, wq_hbm, wkt_hbm, wvt_hbm, woa_hbm, wqkv_hbm, wob_hbm, out_hbm,
            xin_s, wq_in, wkt_in, wvt_in, woa_in, wqkv_in, wob_in, out_s,
            wa_s, woa_s, wb_s, wob_s, xn_s, q_s, ka_s, kb_s, v_s, o_s, p_s, s_s, bound_s,
            qtab_s, ktab0_s, ktab1_s, sems, *bufs):
    xs, pa = bufs[:NT], bufs[NT:]
    ka32, kb32, p32 = ka_s.bitcast(U32), kb_s.bitcast(U32), p_s.bitcast(U32)
    xn32, q32, v32, o32 = (r.bitcast(U32) for r in (xn_s, q_s, v_s, o_s))

    def load_tiles(ref32, tile0, n, row0, rows):
        if isinstance(row0, int):
            sl = slice(row0 // 2, (row0 + rows) // 2)
        else:
            sl = pl.ds(pl.multiple_of(row0 // 2, rows // 2), rows // 2)
        return jnp.concatenate([_unpack(ref32[tile0 + l, sl, :]) for l in range(n)], axis=1)

    def store_tiles(ref, tile0, row0, val):
        if isinstance(row0, int):
            sl = slice(row0, row0 + val.shape[0])
        else:
            sl = pl.ds(pl.multiple_of(row0, val.shape[0]), val.shape[0])
        for l in range(val.shape[1] // 128):
            ref[tile0 + l, sl, :] = val[:, l * 128:(l + 1) * 128].astype(BF16)

    def tok(t):
        return slice(t * BT, (t + 1) * BT)

    x_in = [pltpu.make_async_copy(xt_hbm.at[:, tok(t)], xin_s.at[0:D, tok(t)], sems.at[t])
            for t in range(NT)]
    x_out = [pltpu.make_async_copy(out_s.at[:, tok(t)], out_hbm.at[:, tok(t)], sems.at[NT + t])
             for t in range(NT)]
    w_in = [pltpu.make_async_copy(src, dst, sems.at[2 * NT + n]) for n, (src, dst) in enumerate((
        (wkt_hbm, wkt_in), (wvt_hbm, wvt_in), (wq_hbm, wq_in),
        (woa_hbm, woa_in), (wob_hbm, wob_in), (wqkv_hbm, wqkv_in)))]

    def store_left(dst, r0, lo, hi):
        n = lo.shape[0] // 2
        for i, w in enumerate(_left_operands(lo[:n], hi[:n], lo[n:], hi[n:])):
            w = jnp.concatenate([w, jnp.zeros((n, -w.shape[1] % 128), F32)], axis=1)
            store_tiles(dst, 0, r0 + i * n, w)

    def prep(src, dst):
        for u in range(src.shape[1] // (2 * GR)):
            w = src[:, u * 2 * GR:(u + 1) * 2 * GR].astype(F32)
            lo = w[:D // 2].T
            yield
            store_left(dst, u * 7 * GR, lo, w[D // 2:].T)
            yield

    def prep_kv():
        z = jnp.zeros((HP - DH, D), F32)
        w = jnp.concatenate([wkt_in[...].astype(F32), z, wvt_in[...].astype(F32), z], axis=0)
        store_left(wa_s, 14 * GR, w[:, :D // 2], w[:, D // 2:])

    def prep_wo():
        for src, dst in ((woa_in, woa_s), (wob_in, wob_s)):
            for c in range(0, D, 128):
                w = src[:, c:min(c + 128, D)].astype(F32)
                w = jnp.concatenate([_zero_pad(_head_rows(w, h)) for h in range(H)], axis=0)
                store_tiles(dst, 0, c, w.T)
                yield

    def project(w_s, r0, rows, t, hook):
        def product(i):
            b = load_tiles(xn32, (t * 7 + i) * 2, 2, 0, D // 2)
            y = _dot(load_tiles(w_s.bitcast(U32), 0, 2, r0 + i * rows, rows)[:, 0:D // 2], b)
            hook(y)
            return y
        return _strassen(product)

    def load_x(t):
        moments = _Moments()
        for r in range(0, D, D // 2):
            y = yield
            if y is not None:
                xin_s[pl.ds(pl.multiple_of(D + 16 * zero, 16), 16), 0:128] = (
                    y[0:16, 0:128].astype(xin_s.dtype))
            for c in range(r, r + D // 2, 16):
                x = xin_s[c:c + 16, tok(t)].astype(F32)
                xs[t][c:c + 16, :] = x
                moments.add(x)
        yield from layernorm(t, {t: moments.result()})

    def layernorm(t, stats):
        n = D // 2
        for l in range(2):
            for r in range(0, n, n // 2):
                y = yield
                if y is not None:
                    xs[t][pl.ds(pl.multiple_of(D + 8 * zero, 8), 8), 0:128] = y[0:8, 0:128]
                mean, scale = stats[t]
                for c in range(r, r + n // 2, 16):
                    quarters = []
                    for r0 in (c, n + c):
                        for c0 in (l * 128, (l + 2) * 128):
                            cols = slice(c0, c0 + 128)
                            quarters.append(
                                (xs[t][r0:r0 + 16, cols] - mean[:, cols]) * scale[:, cols])
                    for i, b in enumerate(_right_operands(*quarters)):
                        store_tiles(xn_s, (t * 7 + i) * 2 + l, c, b)
        yield

    def add_out_proj(t, wo_s, hook, emit):
        o = load_tiles(o32, t * NL, NL, 0, DP)
        moments = _Moments()
        for g in range(D // GR):
            y = _dot(load_tiles(wo_s.bitcast(U32), 0, DP // 128, g * GR, GR), o)
            hook(y)
            for c in range(0, GR, 16):
                rows = slice(g * GR + c, g * GR + c + 16)
                x = xs[t][rows, :] + y[c:c + 16]
                xs[t][rows, :] = x
                moments.add(x)
                if emit:
                    out_s[rows, tok(t)] = x.astype(out_s.dtype)
        return moments.result()

    def q_proj(t, u, w_s, hook):
        heads = []
        for g, y in enumerate(project(w_s, u * 7 * GR, GR, t, hook), 2 * u):
            for j in range(4):
                heads.append(_head_rows(y, j) * QSCALE)
                store_tiles(q_s, t * NL, (4 * g + j) * HP, heads[-1])
        return heads

    def project_a(t, hook):
        kt, v = project(wa_s, 14 * GR, HP, t, hook)
        ka_s[tok(t), :] = jnp.concatenate(
            [kt.astype(BF16), jnp.zeros((128 - HP, BT), BF16)], axis=0).T
        v = _ones_pad(v)
        store_tiles(v_s, t * NL, 0, v)
        qq = None
        for u in range(2):
            for q in q_proj(t, u, wa_s, hook):
                n = jnp.sum(q * q, axis=0, keepdims=True)
                qq = n if qq is None else jnp.maximum(qq, n)
        return qq, jnp.sum(kt * kt, axis=0, keepdims=True), _colmax8(jnp.abs(v))

    def store_bounds(bounds):
        for i, b in enumerate(zip(*bounds)):
            b = jnp.concatenate(b, axis=0)
            bound_s[i] = jnp.broadcast_to(jnp.max(b, axis=0, keepdims=True), (8, BT))

    def no_shift_needed():
        qq, kk, vv = (jnp.max(bound_s[i]) for i in range(3))
        return jnp.logical_and(qq * kk <= SCORE_BOUND ** 2, vv <= VALUE_BOUND)

    def store_window_keys(t, g, y, earlier):
        kt = jnp.concatenate([_zero_pad(_head_rows(y, j)) for j in range(4)], axis=0)
        k = pltpu.bitcast(kt.astype(BF16).T, U32)
        n, m = BT // 2, HP // 2
        rolled = [k] + [pltpu.roll(k, HP * s, 1) for s in range(1, 4)]
        before = earlier.get(g, [jnp.zeros((3 * m, 128), U32)] * 4)
        earlier[g] = [x[n - 3 * m:] for x in rolled]
        rolled = [jnp.concatenate(pair, axis=0) for pair in zip(before, rolled)]
        lane = lax.broadcasted_iota(jnp.int32, (n, 128), 1)
        for j in range(4):
            rows = rolled[-j % 4][0:n]
            for lg in range(1, 4):
                rows = jnp.where(lane >= lg * HP, rolled[(lg - j) % 4][lg * m:lg * m + n], rows)
            kb32[4 * g + j, t * n:(t + 1) * n, :] = rows

    def project_b(t, hook, earlier):
        for u in range(2):
            for g, y in enumerate(project(wb_s, (2 + u) * 7 * GR, GR, t, hook), 2 * u):
                store_window_keys(t, g, y, earlier)
            for g, y in enumerate(project(wb_s, (4 + u) * 7 * GR, GR, t, hook), 2 * u):
                for j in range(4):
                    store_tiles(v_s, t * NL, (4 * g + j) * HP, _ones_pad(_head_rows(y, j)))
            q_proj(t, u, wb_s, hook)

    ktabs = (ktab0_s, ktab1_s)
    spare = DH * RV // 8

    def spread_k():
        k = ka_s[0:RV, :].astype(F32)
        for d in range(DH):
            spread = jnp.broadcast_to(k[:, d:d + 1], (RV, 128)).reshape(RV // 8, 8, 128)
            for ktab in ktabs:
                ktab[d * RV // 8:(d + 1) * RV // 8] = spread
            yield

    def load_q(b):
        b = min(b, NB - 1) if isinstance(b, int) else jnp.minimum(b, NB - 1)
        return load_tiles(q32, (b // H) * NL, NL, (b % H) * HP, HP)

    def store_o(b, acc):
        store_tiles(o_s, (b // H) * NL, (b % H) * HP, _normalize(acc))

    def keys(lo, hi):
        return _unpack(ka32[lo // 2:hi // 2, :])[:, 0:HP]

    def put_probs(u, lo, l0, s):
        p = jnp.exp2(s)
        for l in range(s.shape[1] // 128):
            pa[u][l0 + l, lo:lo + s.shape[0], :] = p[:, l * 128:(l + 1) * 128].astype(BF16)

    def stage_q(b):
        q = load_q(b).astype(F32)
        for r in range(HP // 8):
            for l in range(NL):
                ktab0_s[spare + 1 + r * NL + l] = q[r * 8:(r + 1) * 8, l * 128:(l + 1) * 128]

    def spread_q(u, d):
        for l in range(NL):
            q = ktab0_s[spare + 1 + (d // 8) * NL + l]
            qtab_s[(u * DH + d) * NL + l] = jnp.broadcast_to(q[d % 8:d % 8 + 1, :], (8, 128))

    def a_steps(b0, finish, start):
        work = [(u, r0, l0, d) for u in range(UA) for r0 in range(0, RV // 8, VA)
                for l0 in range(0, NL, VL) for d in range(DH)]
        done, batch, dots = 0, 0, None
        for u in range(UA):
            old32 = pa[u].bitcast(U32)
            acc, lo, nd = None, RV, 0
            if start:
                qn = load_q(b0 + u + UA)
                stage_q(b0 + u + UA + 1)
            for c in range(S // 128):
                if finish:
                    p = jnp.concatenate(
                        [_unpack(old32[l, c * 64:(c + 1) * 64, :]) for l in range(NL)], axis=1)
                    part = _dot(load_tiles(v32, c, 1, 0, HP), p)
                    acc = part if acc is None else acc + part
                hi = (c + 1) * 128
                if not start or hi <= lo:
                    continue
                s = _dot(keys(lo, hi), qn)
                for r in range(0, hi - lo, 16):
                    put_probs(u, lo + r, 0, s[r:r + 16])
                    n = lo + r + 16 - RV
                    if n >= 64 and n % 48 == 0 and nd < DH:
                        spread_q((u + 1) % UA, nd)
                        nd += 1
                    due = len(work) * (u * (S - RV) + n) // (UA * (S - RV))
                    if due > done:
                        batch += 1
                        ktabs[batch % 2][spare + zero] = s[r:r + 8, 256:384]
                    while done < due:
                        wu, r0, l0, d = work[done]
                        done += 1
                        qb = jnp.concatenate(
                            [qtab_s[(wu * DH + d) * NL + l0 + l] for l in range(VL)], axis=1)
                        k0 = d * RV // 8 + r0
                        kb = ktabs[batch % 2][k0:k0 + VA].reshape(VA * 8, 128)
                        term = (jnp.concatenate([kb] * VL, axis=1)
                                * jnp.concatenate([qb] * VA, axis=0))
                        dots = term if d == 0 else dots + term
                        if d == DH - 1:
                            put_probs(wu, 8 * r0, l0, dots)
                lo = hi
            if finish:
                store_o(b0 + u, acc)
            assert not start or nd == DH
        assert not start or done == len(work)

    def a_first_steps():
        stage_q(0)
        for d in range(DH):
            spread_q(0, d)
        a_steps(-UA, False, True)

    def a_unshifted():
        def body(i, carry):
            a_steps(i * UA, True, True)
            return carry
        lax.fori_loop(0, NB // UA - 1, body, 0)
        a_steps(NB - UA, True, False)

    def a_shifted():
        def body(b, carry):
            qn = load_q(b)
            m = None
            for c in range(NT):
                s = _dot(keys(c * BT, (c + 1) * BT), qn)
                s_s[tok(c), :] = s
                m = _colmax8(s) if m is None else jnp.maximum(m, _colmax8(s))
            m = jnp.max(m, axis=0, keepdims=True)

            def chunk(c, acc):
                p = jnp.exp2(s_s[pl.ds(pl.multiple_of(c * 256, 256), 256), :] - m).astype(BF16)
                return acc + _dot(load_tiles(v32, 2 * c, 2, 0, HP), p)

            store_o(b, lax.fori_loop(0, S // 256, chunk, jnp.zeros((HP, BT), F32)))
            return carry
        lax.fori_loop(0, NB, body, 0)

    nb = W // HP

    def b_scores(i, h):
        row = lax.broadcasted_iota(jnp.int32, (HP, QT), 0)
        col = lax.broadcasted_iota(jnp.int32, (HP, QT), 1)
        q = load_tiles(q32, i, 1, h * HP, HP).astype(F32)
        rhs = jnp.concatenate([jnp.where(col >> 5 == lg, q, 0.0) for lg in range(4)], axis=0)
        first = max(0, nb - 4 * i - 3)
        r0 = i * QT - W + first * HP + 3 * HP
        s = _dot(_unpack(kb32[h, r0 // 2:(r0 + (nb + 1 - first) * HP) // 2, :]), rhs.astype(BF16))
        blk = {n: s[(n - first) * HP:(n - first + 1) * HP] for n in range(first, nb + 1)}
        for n in range(first, nb - 4 * i):
            blk[n] = jnp.where((col >> 5) + n >= nb - 4 * i, blk[n], -jnp.inf)
        blk[nb] = jnp.where(row > (col & 31), blk.pop(0) if first == 0 else -jnp.inf, blk[nb])
        m = None
        for x in blk.values():
            m = _colmax8(x) if m is None else jnp.maximum(m, _colmax8(x))
        return blk, jnp.max(m, axis=0, keepdims=True)

    def b_finish(i, h, blk, m):
        p = {n: jnp.exp2(x - m) for n, x in blk.items()}
        if 4 * i >= nb:
            row = lax.broadcasted_iota(jnp.int32, (HP, QT), 0)
            old = row > (lax.broadcasted_iota(jnp.int32, (HP, QT), 1) & 31)
            p[0] = jnp.where(old, p[nb], 0.0)
            p[nb] = jnp.where(old, 0.0, p[nb])
        for n, x in p.items():
            p_s[h, n * HP:(n + 1) * HP, :] = x.astype(BF16)
        p = {n: p32[h, n * HP // 2:(n + 1) * HP // 2, :] for n in p}
        none = jnp.zeros((HP // 2, QT), U32)
        col = lax.broadcasted_iota(jnp.int32, (HP // 2, QT), 1)
        lo = max(0, nb - 4 * i)
        c = {n: jnp.where(col & HP != 0, p.get(n - 1, none), p.get(n, none))
             for n in range(max(0, lo - 2), nb + 2)}
        u = [jnp.where(col & (2 * HP) != 0, c.get(n - 2, none), c.get(n, none))
             for n in range(lo, nb + 4)]
        tiles = (nb + 4 - lo) // 4
        acc = _dot(load_tiles(v32, i + 1 - tiles, tiles, h * HP, HP),
                   _unpack(jnp.concatenate(u, axis=0)))
        store_tiles(o_s, i, h * HP, _normalize(acc))

    def b_attention():
        pending = []
        for i in TILE_ORDER:
            for h in range(H):
                pending.append((i, h) + b_scores(i, h))
                if len(pending) > DB:
                    b_finish(*pending.pop(0))
                yield
        while pending:
            b_finish(*pending.pop(0))
            yield

    def add_attention(wo_s, jobs, emit):
        stats = {}
        ln = layernorm(0, stats)
        next(ln)
        for t in range(NT):
            at = ((), (0, 2), (0,), (0,))[t]
            hook = _paced(*jobs[t], *([(_forward(ln), at)] if at else []))
            stats[t] = add_out_proj(t, wo_s, hook, emit)
            if emit:
                for cp in ([], [], x_out[:3], x_out[3:])[t]:
                    cp.start()
        return stats

    def next_layernorm(t, stats, at):
        return [(layernorm(t + 1, stats), at)] if t + 1 < NT else []

    for cp in x_in[:1] + w_in[:3]:
        cp.start()
    x_in[0].wait()
    for cp in x_in[1:]:
        cp.start()
    _run(load_x(0))
    for cp in w_in[:3]:
        cp.wait()
    for cp in w_in[3:]:
        cp.start()
    zero = jnp.minimum(jnp.max(pltpu.bitcast(jnp.abs(wkt_in[0:16, :].astype(F32)), jnp.int32)), 0)
    prep_kv()
    first_keys, first_bounds = spread_k(), []
    for t in range(NT):
        for cp in (x_in[1:2], x_in[2:], [], w_in[3:5])[t]:
            cp.wait()
        one = ((_pieces(prep(wq_in, wa_s), 2), (0, 7)) if t == 0 else
               (_pieces(first_keys, 1), range(0, 21, 4) if t + 1 < NT else range(16)))
        two = ((load_x(t + 1), (2, 5, 8, 11, 14, 16)) if t + 1 < NT else
               (_pieces(prep_wo(), 1), range(1, 17, 2)))
        first_bounds.append(project_a(t, _paced(one, two)))
    _run(first_keys)
    store_bounds(first_bounds)
    w_in[5].wait()

    def layer_pair(l, carry):
        safe = no_shift_needed()
        a_first_steps()
        lax.cond(safe, a_unshifted, a_shifted)
        weights = prep(wqkv_in, wb_s)
        stats = add_attention(woa_s, [[(_pieces(weights, 1), range(4))] for _ in range(NT)], False)
        _run(weights)
        earlier = {}
        for t in range(NT):
            project_b(t, _paced(*next_layernorm(t, stats, (7, 14, 28, 35))), earlier)
        window = b_attention()
        for _ in range(H * S // QT + DB - 8):
            next(window)
        stats = add_attention(wob_s, [[(_pieces(window, 2), range(4))], [], [], []], True)

        @pl.when(l == 0)
        def _():
            spread, bounds = spread_k(), []
            for t in range(NT):
                at = ((), range(14, 21), range(14, 21), range(14))[t]
                bounds.append(project_a(t, _paced(
                    (_pieces(spread, 1), at), *next_layernorm(t, stats, (1, 4, 8, 12)))))
            _run(spread)
            for cp in x_out:
                cp.wait()
            store_bounds(bounds)

        return carry

    lax.fori_loop(0, 2, layer_pair, 0)
    for cp in x_out:
        cp.wait()


@jax.jit
def pallas_interleave_layers__grouped_kv_mqa__sliding_block__prompt_kernel(
    A_x: jax.Array,
    A_wq: jax.Array,
    A_wk: jax.Array,
    A_wv: jax.Array,
    A_wo: jax.Array,
    B_x: jax.Array,
    B_wqkv: jax.Array,
    B_wo: jax.Array,
):
    del B_x
    operands = (A_x[0].T, A_wq, A_wk.T, A_wv.T, A_wo, B_wqkv, B_wo)
    scratch = [pltpu.VMEM((D + 16, S), A_x.dtype)]
    scratch += [pltpu.VMEM(a.shape, a.dtype) for a in operands[1:]]
    scratch += [
        pltpu.VMEM((D, S), A_x.dtype),
        pltpu.VMEM((2, 14 * GR + 7 * HP, 128), BF16),
        pltpu.VMEM((4, D, 128), BF16),
        pltpu.VMEM((2, 42 * GR, 128), BF16),
        pltpu.VMEM((4, D, 128), BF16),
        pltpu.VMEM((NT * 14, D // 2, 128), BF16),
        pltpu.VMEM((S // 128, DP, 128), BF16),
        pltpu.VMEM((S, 128), BF16),
        pltpu.VMEM((H, S, 128), BF16),
        pltpu.VMEM((S // 128, DP, 128), BF16),
        pltpu.VMEM((S // 128, DP, 128), BF16),
        pltpu.VMEM((H, W + HP, QT), BF16),
        pltpu.VMEM((S, BT), F32),
        pltpu.VMEM((3, 8, BT), F32),
        pltpu.VMEM((UA * DH * NL, 8, 128), F32),
        pltpu.VMEM((DH * RV // 8 + 1 + HP // 8 * NL, 8, 128), F32),
        pltpu.VMEM((DH * RV // 8 + 1, 8, 128), F32),
        pltpu.SemaphoreType.DMA((2 * NT + 6,)),
    ]
    scratch += [pltpu.VMEM((D + 8, BT), F32)] * NT
    scratch += [pltpu.VMEM((NL, S, 128), BF16)] * UA
    out_t = pl.pallas_call(
        _kernel,
        out_shape=jax.ShapeDtypeStruct((D, S), A_x.dtype),
        in_specs=[pl.BlockSpec(memory_space=pl.ANY)] * len(operands),
        out_specs=pl.BlockSpec(memory_space=pl.ANY),
        scratch_shapes=scratch,
        compiler_params=pltpu.CompilerParams(vmem_limit_bytes=100 * 1024 * 1024),
        name="interleave_layers",
    )(*operands)
    return out_t.T[None]
```
